```python
import os as _os
_os.environ.setdefault("JAX_PLATFORMS", "cpu")
import jax
import jax.numpy as jnp

def _softmax(x, axis=-1):
    return jax.nn.softmax(x, axis=axis)
def _gelu(x):
    return jax.nn.gelu(x, approximate=True)
def _silu(x):
    return jax.nn.silu(x)
def _sigmoid(x):
    return jax.nn.sigmoid(x)
def _layernorm(x, axis=-1, eps=1e-5):
    m = jnp.mean(x, axis=axis, keepdims=True)
    v = jnp.var(x, axis=axis, keepdims=True)
    return (x - m) / jnp.sqrt(v + eps)
def _scatter_add(tgt, idx, src, axis=0):
    return tgt.at[idx].add(src)
def _segment_sum(src, seg, n):
    return jax.ops.segment_sum(src, seg, n)
class _Rng:
    def __init__(self, key):
        self._k = key
    def _next(self):
        self._k, sub = jax.random.split(self._k)
        return sub
    def normal(self, shape):
        return jax.random.normal(self._next(), shape, dtype=jnp.bfloat16)
    def randint(self, lo, hi, shape):
        return jax.random.randint(self._next(), shape, lo, hi, dtype=jnp.int32)
    def uniform(self, shape, lo=0.0, hi=1.0):
        return jax.random.uniform(self._next(), shape, jnp.bfloat16, lo, hi)
    def permutation(self, n):
        return jax.random.permutation(self._next(), n)


kernel_name = 'standalone__gqa_block_cached__near_ridge'

def setup_inputs():
    _rng = _Rng(jax.random.key(int.from_bytes(__import__("os").urandom(4), "little")))
    _w = (lambda a: (lambda t: t.astype(jnp.bfloat16) if jnp.issubdtype(t.dtype, jnp.floating) else t)(jnp.asarray(a)))
    B, Sq, D = 8, 64, 512
    Hq, Hkv, Sk, Dh = 32, 8, 64, 128
    assert Hq % Hkv == 0, (Hq, Hkv)
    return {
        "x": _w((lambda *s: _rng.normal(s) * 0.8)(B, Sq, D)),
        "k_cache": _w((lambda *s: _rng.normal(s) * 0.8)(B, Hkv, Sk, Dh)),
        "v_cache": _w((lambda *s: _rng.normal(s) * 0.05)(B, Hkv, Sk, Dh)),
        "wq": _w((lambda *s: _rng.normal(s) * 0.8)(D, Hq * Dh) * (D ** -0.5)),
        "wo": _w((lambda *s: _rng.normal(s) * 0.05)(Hq * Dh, D) * ((Hq * Dh) ** -0.5)),
    }

def reference(x, k_cache, v_cache, wq, wo):
    B, Sq, D = x.shape
    Hq, Dh = 32, 128
    Hkv = k_cache.shape[1]
    rep = Hq // Hkv
    q = (lambda x, *d: x.transpose(*d))((x @ wq).reshape(B, Sq, Hq, Dh), 0, 2, 1, 3)
    k = jnp.repeat(k_cache, rep, axis=1)
    v = jnp.repeat(v_cache, rep, axis=1)
    scores = jnp.einsum("bhqd,bhkd->bhqk", q, k) * (Dh ** -0.5)
    p = _softmax(scores, axis=-1)
    o = jnp.einsum("bhqk,bhkd->bhqd", p, v)
    return (lambda x, *d: x.transpose(*d))(o, 0, 2, 1, 3).reshape(B, Sq, Hq * Dh) @ wo
```

```python
import functools

import jax
import jax.numpy as jnp
from jax import lax
import jax.experimental.pallas as pl
import jax.experimental.pallas.tpu as pltpu

_F32 = jnp.float32
_BF16 = jnp.bfloat16
_LOG2E = 1.4426950408889634
_NSUB = 4
_OUT_ROWS = 64
_WAIT_BEFORE = (("sd", 0, 0), ("sd", 1, 0), ("sd", 2, 0), ("sd", 4, 0))


def _phases(G):
    ph = [("qp", 0, j) for j in range(_NSUB)]
    for g in range(G):
        for j in range(_NSUB):
            ph.append(("sd", g, j))
            if g + 1 < G:
                ph += [("qp", g + 1, j), ("pv", g, j)]
                if g > 0:
                    ph.append(("op", g - 1, j))
            else:
                ph += [("op", g - 1, j), ("pv", g, j)]
    ph.append(("last", G - 1, 0))
    return ph


def _needs(ph):
    t, g, _ = ph
    return {"qp": [("x", 0), ("wq", g)], "sd": [("k", g)], "pv": [("v", g)],
            "op": [("wo", g)], "last": [("wo", g)]}[t]


def _kernel(x_hbm, k_hbm, v_hbm, wq_hbm, wo_hbm, o_hbm,
            x_buf, k_buf, v_buf, wq_buf, wo_buf, q_buf, att_buf, acc_ref, o_buf, sems,
            *, B, Sq, rep, Dh, G, scale):
    C = rep * Dh
    T, D = x_buf.shape
    bps = B // _NSUB
    hps = rep // _NSUB
    nps = D // _NSUB

    phases = _phases(G)
    groups, seen = [], set()
    for i, ph in enumerate(phases):
        if i == 0 or ph in _WAIT_BEFORE:
            groups.append([])
        for n in _needs(ph):
            if n not in seen:
                seen.add(n)
                groups[-1].append(n)
    gid = {n: gi for gi, grp in enumerate(groups) for n in grp}
    out_sem = len(groups)
    out_pieces = [(lo, lo + _OUT_ROWS) for lo in range(0, T, _OUT_ROWS)]

    def copy_in(name, g):
        sem = sems.at[gid[(name, g)]]
        if name == "x":
            return pltpu.make_async_copy(x_hbm, x_buf, sem)
        if name == "wq":
            return pltpu.make_async_copy(wq_hbm.at[:, pl.ds(g * C, C)], wq_buf.at[g], sem)
        if name == "wo":
            return pltpu.make_async_copy(wo_hbm.at[pl.ds(g * C, C), :], wo_buf.at[g], sem)
        if name == "k":
            return pltpu.make_async_copy(k_hbm.at[:, g], k_buf.at[g], sem)
        return pltpu.make_async_copy(v_hbm.at[:, g], v_buf.at[g], sem)

    def copy_out(i):
        lo, hi = out_pieces[i]
        return pltpu.make_async_copy(
            o_buf.at[pl.ds(lo, hi - lo), :], o_hbm.at[pl.ds(lo, hi - lo), :], sems.at[out_sem])

    def qp(g, j):
        lo, hi = j * hps * Dh, (j + 1) * hps * Dh
        q = jnp.dot(x_buf[...], wq_buf[g, :, lo:hi], preferred_element_type=_F32)
        q_buf[g % 2, :, lo:hi] = q.astype(_BF16)

    def sd(g, j):
        out = []
        for b in range(j * bps, (j + 1) * bps):
            qb = jnp.concatenate(
                [q_buf[g % 2, b * Sq:(b + 1) * Sq, h * Dh:(h + 1) * Dh] for h in range(rep)], axis=0)
            out.append(lax.dot_general(k_buf[g, b], qb, (((1,), (1,)), ((), ())),
                                       preferred_element_type=_F32))
        return out

    def pv(g, j, scores_t):
        for s, b in zip(scores_t, range(j * bps, (j + 1) * bps)):
            m = jnp.max(s, axis=0, keepdims=True)
            e = jnp.exp2((s - m) * (scale * _LOG2E))
            p_t = (e / jnp.sum(e, axis=0, keepdims=True)).astype(_BF16)
            o = lax.dot_general(p_t, v_buf[g, b], (((0,), (0,)), ((), ())),
                                preferred_element_type=_F32).astype(_BF16)
            for h in range(rep):
                att_buf[g % 2, b * Sq:(b + 1) * Sq, h * Dh:(h + 1) * Dh] = o[h * Sq:(h + 1) * Sq]

    def op(g, j):
        lo, hi = j * nps, (j + 1) * nps
        contrib = jnp.dot(att_buf[g % 2], wo_buf[g, :, lo:hi], preferred_element_type=_F32)
        if g == 0:
            acc_ref[:, lo:hi] = contrib
        else:
            acc_ref[:, lo:hi] += contrib

    def last(g):
        for i, (lo, hi) in enumerate(out_pieces):
            contrib = jnp.dot(att_buf[g % 2, lo:hi, :], wo_buf[g], preferred_element_type=_F32)
            o_buf[lo:hi, :] = (acc_ref[lo:hi, :] + contrib).astype(o_buf.dtype)
            copy_out(i).start()

    for grp in groups:
        for n in grp:
            copy_in(*n).start()

    scores = {}
    next_group = 0
    for i, ph in enumerate(phases):
        if i == 0 or ph in _WAIT_BEFORE:
            for n in groups[next_group]:
                copy_in(*n).wait()
            next_group += 1
        t, g, j = ph
        if t == "qp":
            qp(g, j)
        elif t == "sd":
            scores[g, j] = sd(g, j)
        elif t == "pv":
            pv(g, j, scores.pop((g, j)))
        elif t == "op":
            op(g, j)
        else:
            last(g)

    for i in range(len(out_pieces)):
        copy_out(i).wait()


@jax.jit
def pallas_standalone__gqa_block_cached__near_ridge_kernel(
    x: jax.Array,
    k_cache: jax.Array,
    v_cache: jax.Array,
    wq: jax.Array,
    wo: jax.Array,
):
    B, Sq, D = x.shape
    _, Hkv, Sk, Dh = k_cache.shape
    Hq = wq.shape[1] // Dh
    rep = Hq // Hkv
    C = rep * Dh
    T = B * Sq
    hbm = pl.BlockSpec(memory_space=pl.ANY)
    out = pl.pallas_call(
        functools.partial(_kernel, B=B, Sq=Sq, rep=rep, Dh=Dh, G=Hkv, scale=Dh ** -0.5),
        in_specs=[hbm] * 5,
        out_specs=hbm,
        out_shape=jax.ShapeDtypeStruct((T, D), x.dtype),
        scratch_shapes=[
            pltpu.VMEM((T, D), x.dtype),
            pltpu.VMEM((Hkv, B, Sk, Dh), k_cache.dtype),
            pltpu.VMEM((Hkv, B, Sk, Dh), v_cache.dtype),
            pltpu.VMEM((Hkv, D, C), wq.dtype),
            pltpu.VMEM((Hkv, C, D), wo.dtype),
            pltpu.VMEM((2, T, C), _BF16),
            pltpu.VMEM((2, T, C), _BF16),
            pltpu.VMEM((T, D), _F32),
            pltpu.VMEM((T, D), x.dtype),
            pltpu.SemaphoreType.DMA((len(_WAIT_BEFORE) + 2,)),
        ],
        compiler_params=pltpu.CompilerParams(vmem_limit_bytes=48 * 1024 * 1024),
        name="gqa_block_cached",
    )(x.reshape(T, D), k_cache, v_cache, wq, wo)
    return out.reshape(B, Sq, D)
```

```python
import functools

import jax
import jax.numpy as jnp
from jax import lax
import jax.experimental.pallas as pl
import jax.experimental.pallas.tpu as pltpu

_F32 = jnp.float32
_LOG2E = 1.4426950408889634
_SLOTS = 4
_OUT_ROWS = (128, 128, 64, 64, 64, 32, 32)
_NUM_WAITS = 6


def _kernel(x_hbm, k_hbm, v_hbm, wq_hbm, wo_hbm, o_hbm,
            x_buf, k_buf, v_buf, wq_buf, wo_buf, q_buf, att_buf, acc_ref, o_buf, sems,
            *, B, Sq, rep, Dh, G, scale):
    T, D = x_buf.shape
    C = rep * Dh
    half = T // 2
    bps = B // _SLOTS
    nps = D // _SLOTS
    assert G == 8 and rep == _SLOTS and sum(_OUT_ROWS) == T

    def cp_x(s, r0, r1):
        r = pl.ds(r0, r1 - r0)
        return pltpu.make_async_copy(x_hbm.at[r, :], x_buf.at[r, :], sems.at[s])

    def cp_wq(s, g, h0=0, h1=rep):
        n = (h1 - h0) * Dh
        return pltpu.make_async_copy(wq_hbm.at[:, pl.ds(g * C + h0 * Dh, n)],
                                     wq_buf.at[g, :, pl.ds(h0 * Dh, n)], sems.at[s])

    def cp_wo(s, g0, g1):
        r = pl.ds(g0 * C, (g1 - g0) * C)
        return pltpu.make_async_copy(wo_hbm.at[r, :], wo_buf.at[r, :], sems.at[s])

    def cp_kv(src, dst, s, g0, g1, b0=0, b1=B):
        b, g = pl.ds(b0, b1 - b0), pl.ds(g0, g1 - g0)
        return pltpu.make_async_copy(src.at[b, g], dst.at[b, g], sems.at[s])

    cp_k = functools.partial(cp_kv, k_hbm, k_buf)
    cp_v = functools.partial(cp_kv, v_hbm, v_buf)

    def cp_o(i):
        r = pl.ds(sum(_OUT_ROWS[:i]), _OUT_ROWS[i])
        return pltpu.make_async_copy(o_buf.at[r, :], o_hbm.at[r, :], sems.at[_NUM_WAITS])

    groups = [
        [cp_wq(0, 0, 0, rep - 1), cp_x(0, 0, half)],
        [cp_x(1, half, T), cp_wq(1, 0, rep - 1, rep)],
        [cp_k(2, 0, 1), cp_wq(2, 1), cp_v(2, 0, 1), cp_k(2, 1, 2, 0, bps)],
        [cp_wq(3, 2), cp_v(3, 1, 2), cp_wo(3, 0, 1), cp_k(3, 1, 2, bps, B), cp_k(3, 2, 3, 0, bps)],
        [cp_wq(4, 3), cp_v(4, 2, 4), cp_wo(4, 1, 3), cp_k(4, 2, 3, bps, B), cp_k(4, 3, 4),
         cp_wq(4, 4), cp_k(4, 4, 5, 0, bps)],
        [cp_wq(5, 5), cp_v(5, 4, 8), cp_wo(5, 3, 8), cp_k(5, 4, 5, bps, B), cp_k(5, 5, 8),
         cp_wq(5, 6), cp_wq(5, 7)],
    ]
    wait_after_first_scores = {1: 3, 2: 4, 4: 5}

    def wait(s):
        for c in groups[s]:
            c.wait()

    def q_proj(g, h, r0=0, r1=T):
        cols = slice(h * Dh, (h + 1) * Dh)
        q = jnp.dot(x_buf[r0:r1, :], wq_buf[g, :, cols], preferred_element_type=_F32)
        q_buf[g % 2, r0:r1, cols] = q.astype(q_buf.dtype)

    def scores_t(g, b):
        rows = slice(b * Sq, (b + 1) * Sq)
        q = jnp.concatenate(
            [q_buf[g % 2, rows, h * Dh:(h + 1) * Dh] for h in range(rep)], axis=0)
        return lax.dot_general(k_buf[b, g], q, (((1,), (1,)), ((), ())),
                               preferred_element_type=_F32)

    def softmax_pv(g, b, s):
        m = jnp.max(s, axis=0, keepdims=True)
        e = jnp.exp2((s - m) * (scale * _LOG2E))
        p_t = (e / jnp.sum(e, axis=0, keepdims=True)).astype(v_buf.dtype)
        o = lax.dot_general(p_t, v_buf[b, g], (((0,), (0,)), ((), ())),
                            preferred_element_type=_F32).astype(att_buf.dtype)
        for h in range(rep):
            att_buf[g % 2, b * Sq:(b + 1) * Sq, h * Dh:(h + 1) * Dh] = o[h * Sq:(h + 1) * Sq]

    def out_proj(g, j):
        cols = slice(j * nps, (j + 1) * nps)
        contrib = jnp.dot(att_buf[g % 2], wo_buf[g * C:(g + 1) * C, cols],
                          preferred_element_type=_F32)
        if g == 0:
            acc_ref[:, cols] = contrib
        else:
            acc_ref[:, cols] += contrib

    for grp in groups:
        for c in grp:
            c.start()

    wait(0)
    for h in range(rep - 1):
        q_proj(0, h, 0, half)
    wait(1)
    q_proj(0, rep - 1, 0, half)
    for h in range(rep):
        q_proj(0, h, half, T)
    wait(2)

    for g in range(G):
        for j in range(_SLOTS):
            batches = range(j * bps, (j + 1) * bps)
            scores = [scores_t(g, b) for b in batches]
            if j == 0 and g in wait_after_first_scores:
                wait(wait_after_first_scores[g])
            if g + 1 < G:
                q_proj(g + 1, j)
            else:
                out_proj(g - 1, j)
            for b, s in zip(batches, scores):
                softmax_pv(g, b, s)
            if 0 < g < G - 1:
                out_proj(g - 1, j)

    g = G - 1
    r0 = 0
    for i, n in enumerate(_OUT_ROWS):
        rows = slice(r0, r0 + n)
        contrib = jnp.dot(att_buf[g % 2, rows, :], wo_buf[g * C:(g + 1) * C, :],
                          preferred_element_type=_F32)
        o_buf[rows, :] = (acc_ref[rows, :] + contrib).astype(o_buf.dtype)
        cp_o(i).start()
        r0 += n
    for i in range(len(_OUT_ROWS)):
        cp_o(i).wait()


@jax.jit
def pallas_standalone__gqa_block_cached__near_ridge_kernel(
    x: jax.Array,
    k_cache: jax.Array,
    v_cache: jax.Array,
    wq: jax.Array,
    wo: jax.Array,
):
    B, Sq, D = x.shape
    _, Hkv, Sk, Dh = k_cache.shape
    Hq = wq.shape[1] // Dh
    rep = Hq // Hkv
    C = rep * Dh
    T = B * Sq
    hbm = pl.BlockSpec(memory_space=pl.ANY)
    out = pl.pallas_call(
        functools.partial(_kernel, B=B, Sq=Sq, rep=rep, Dh=Dh, G=Hkv, scale=Dh ** -0.5),
        in_specs=[hbm] * 5,
        out_specs=hbm,
        out_shape=jax.ShapeDtypeStruct((T, D), x.dtype),
        scratch_shapes=[
            pltpu.VMEM((T, D), x.dtype),
            pltpu.VMEM((B, Hkv, Sk, Dh), k_cache.dtype),
            pltpu.VMEM((B, Hkv, Sk, Dh), v_cache.dtype),
            pltpu.VMEM((Hkv, D, C), wq.dtype),
            pltpu.VMEM((Hq * Dh, D), wo.dtype),
            pltpu.VMEM((2, T, C), x.dtype),
            pltpu.VMEM((2, T, C), x.dtype),
            pltpu.VMEM((T, D), _F32),
            pltpu.VMEM((T, D), x.dtype),
            pltpu.SemaphoreType.DMA((_NUM_WAITS + 1,)),
        ],
        compiler_params=pltpu.CompilerParams(vmem_limit_bytes=48 * 1024 * 1024),
        name="gqa_block_cached",
    )(x.reshape(T, D), k_cache, v_cache, wq, wo)
    return out.reshape(B, Sq, D)
```

```python
import functools

import jax
import jax.numpy as jnp
from jax import lax
import jax.experimental.pallas as pl
import jax.experimental.pallas.tpu as pltpu

_F32 = jnp.float32
_LOG2E = 1.4426950408889634
_SLOTS = 4
_OUT_ROWS = (128, 128, 64, 64, 64, 32, 32)
_NUM_WAITS = 6


def _kernel(x_hbm, k_hbm, v_hbm, wq_hbm, wo_hbm, o_hbm,
            x_buf, k_buf, v_buf, wq_buf, wo_buf, acc_ref, o_buf, sems,
            *, B, Sq, rep, Dh, G, scale):
    T, D = x_buf.shape
    C = rep * Dh
    half = T // 2
    bps = B // _SLOTS
    nps = D // _SLOTS
    dt = x_buf.dtype
    assert G == 8 and rep == _SLOTS and sum(_OUT_ROWS) == T

    def cp_x(s, r0, r1):
        r = pl.ds(r0, r1 - r0)
        return pltpu.make_async_copy(x_hbm.at[r, :], x_buf.at[r, :], sems.at[s])

    def cp_wq(s, g, h0=0, h1=rep):
        n = (h1 - h0) * Dh
        return pltpu.make_async_copy(wq_hbm.at[:, pl.ds(g * C + h0 * Dh, n)],
                                     wq_buf.at[g, :, pl.ds(h0 * Dh, n)], sems.at[s])

    def cp_wo(s, g0, g1):
        r = pl.ds(g0 * C, (g1 - g0) * C)
        return pltpu.make_async_copy(wo_hbm.at[r, :], wo_buf.at[r, :], sems.at[s])

    def cp_kv(src, dst, s, g0, g1, b0=0, b1=B):
        b, g = pl.ds(b0, b1 - b0), pl.ds(g0, g1 - g0)
        return pltpu.make_async_copy(src.at[b, g], dst.at[b, g], sems.at[s])

    cp_k = functools.partial(cp_kv, k_hbm, k_buf)
    cp_v = functools.partial(cp_kv, v_hbm, v_buf)

    def cp_o(i):
        r = pl.ds(sum(_OUT_ROWS[:i]), _OUT_ROWS[i])
        return pltpu.make_async_copy(o_buf.at[r, :], o_hbm.at[r, :], sems.at[_NUM_WAITS])

    groups = [
        [cp_wq(0, 0, 0, rep - 1), cp_x(0, 0, half)],
        [cp_x(1, half, T), cp_wq(1, 0, rep - 1, rep)],
        [cp_k(2, 0, 1), cp_wq(2, 1), cp_v(2, 0, 1), cp_k(2, 1, 2, 0, bps)],
        [cp_wq(3, 2), cp_v(3, 1, 2), cp_wo(3, 0, 1), cp_k(3, 1, 2, bps, B), cp_k(3, 2, 3, 0, bps)],
        [cp_wq(4, 3), cp_v(4, 2, 4), cp_wo(4, 1, 3), cp_k(4, 2, 3, bps, B), cp_k(4, 3, 4),
         cp_wq(4, 4), cp_k(4, 4, 5, 0, bps)],
        [cp_wq(5, 5), cp_v(5, 4, 8), cp_wo(5, 3, 8), cp_k(5, 4, 5, bps, B), cp_k(5, 5, 8),
         cp_wq(5, 6), cp_wq(5, 7)],
    ]
    wait_after_first_scores = {1: 3, 2: 4, 4: 5}

    def wait(s):
        for c in groups[s]:
            c.wait()

    q = {}
    att = {}

    def q_proj(g, h, xs, b0):
        qh = jnp.dot(xs, wq_buf[g, :, h * Dh:(h + 1) * Dh], preferred_element_type=_F32).astype(dt)
        for i in range(xs.shape[0] // Sq):
            q[g, h, b0 + i] = qh[i * Sq:(i + 1) * Sq]

    def scores_t(g, b):
        qb = jnp.concatenate([q.pop((g, h, b)) for h in range(rep)], axis=0)
        return lax.dot_general(k_buf[b, g], qb, (((1,), (1,)), ((), ())),
                               preferred_element_type=_F32)

    def softmax_pv(g, b, s):
        m = jnp.max(s, axis=0, keepdims=True)
        e = jnp.exp2((s - m) * (scale * _LOG2E))
        p_t = (e / jnp.sum(e, axis=0, keepdims=True)).astype(dt)
        o = lax.dot_general(p_t, v_buf[b, g], (((0,), (0,)), ((), ())),
                            preferred_element_type=_F32).astype(dt)
        for h in range(rep):
            att[g, b, h] = o[h * Sq:(h + 1) * Sq]

    def att_of(g):
        if g not in att:
            att[g] = jnp.concatenate(
                [jnp.concatenate([att.pop((g, b, h)) for h in range(rep)], axis=1)
                 for b in range(B)], axis=0)
        return att[g]

    def out_proj(g, j):
        cols = slice(j * nps, (j + 1) * nps)
        contrib = jnp.dot(att_of(g), wo_buf[g * C:(g + 1) * C, cols], preferred_element_type=_F32)
        if g == 0:
            acc_ref[:, cols] = contrib
        else:
            acc_ref[:, cols] += contrib

    for grp in groups:
        for c in grp:
            c.start()

    wait(0)
    x_lo = x_buf[:half, :]
    for h in range(rep - 1):
        q_proj(0, h, x_lo, 0)
    wait(1)
    x_hi = x_buf[half:, :]
    q_proj(0, rep - 1, x_lo, 0)
    for h in range(rep):
        q_proj(0, h, x_hi, B // 2)
    x = jnp.concatenate([x_lo, x_hi], axis=0)
    wait(2)

    for g in range(G):
        for j in range(_SLOTS):
            batches = range(j * bps, (j + 1) * bps)
            scores = [scores_t(g, b) for b in batches]
            if j == 0 and g in wait_after_first_scores:
                wait(wait_after_first_scores[g])
            if g + 1 < G:
                q_proj(g + 1, j, x, 0)
            else:
                out_proj(g - 1, j)
            for b, s in zip(batches, scores):
                softmax_pv(g, b, s)
            if 0 < g < G - 1:
                out_proj(g - 1, j)

    g = G - 1
    r0 = 0
    for i, n in enumerate(_OUT_ROWS):
        rows = slice(r0, r0 + n)
        contrib = jnp.dot(att_of(g)[rows], wo_buf[g * C:(g + 1) * C, :],
                          preferred_element_type=_F32)
        o_buf[rows, :] = (acc_ref[rows, :] + contrib).astype(o_buf.dtype)
        cp_o(i).start()
        r0 += n
    for i in range(len(_OUT_ROWS)):
        cp_o(i).wait()


@jax.jit
def pallas_standalone__gqa_block_cached__near_ridge_kernel(
    x: jax.Array,
    k_cache: jax.Array,
    v_cache: jax.Array,
    wq: jax.Array,
    wo: jax.Array,
):
    B, Sq, D = x.shape
    _, Hkv, Sk, Dh = k_cache.shape
    Hq = wq.shape[1] // Dh
    rep = Hq // Hkv
    C = rep * Dh
    T = B * Sq
    hbm = pl.BlockSpec(memory_space=pl.ANY)
    out = pl.pallas_call(
        functools.partial(_kernel, B=B, Sq=Sq, rep=rep, Dh=Dh, G=Hkv, scale=Dh ** -0.5),
        in_specs=[hbm] * 5,
        out_specs=hbm,
        out_shape=jax.ShapeDtypeStruct((T, D), x.dtype),
        scratch_shapes=[
            pltpu.VMEM((T, D), x.dtype),
            pltpu.VMEM((B, Hkv, Sk, Dh), k_cache.dtype),
            pltpu.VMEM((B, Hkv, Sk, Dh), v_cache.dtype),
            pltpu.VMEM((Hkv, D, C), wq.dtype),
            pltpu.VMEM((Hq * Dh, D), wo.dtype),
            pltpu.VMEM((T, D), _F32),
            pltpu.VMEM((T, D), x.dtype),
            pltpu.SemaphoreType.DMA((_NUM_WAITS + 1,)),
        ],
        compiler_params=pltpu.CompilerParams(vmem_limit_bytes=48 * 1024 * 1024),
        name="gqa_block_cached",
    )(x.reshape(T, D), k_cache, v_cache, wq, wo)
    return out.reshape(B, Sq, D)
```

```python
import functools

import jax
import jax.numpy as jnp
from jax import lax
import jax.experimental.pallas as pl
import jax.experimental.pallas.tpu as pltpu

_F32 = jnp.float32
_LOG2E = 1.4426950408889634
_SLOTS = 4
_OUT_ROWS = (128, 128, 64, 64, 64, 32, 32)
_NUM_WAITS = 6


def _kernel(x_hbm, k_hbm, v_hbm, wq_hbm, wo_hbm, o_hbm,
            x_buf, k_buf, v_buf, wq_buf, wo_buf, acc_ref, o_buf, trips_ref, sems,
            *, B, Sq, rep, Dh, G, scale):
    T, D = x_buf.shape
    C = rep * Dh
    half = T // 2
    bps = B // _SLOTS
    nps = D // _SLOTS
    dt = x_buf.dtype
    assert G == 8 and rep == _SLOTS and sum(_OUT_ROWS) == T

    def cp_x(s, r0, r1):
        r = pl.ds(r0, r1 - r0)
        return pltpu.make_async_copy(x_hbm.at[r, :], x_buf.at[r, :], sems.at[s])

    def cp_wq(s, g, h0=0, h1=rep):
        n = (h1 - h0) * Dh
        return pltpu.make_async_copy(wq_hbm.at[:, pl.ds(g * C + h0 * Dh, n)],
                                     wq_buf.at[g, :, pl.ds(h0 * Dh, n)], sems.at[s])

    def cp_wo(s, g0, g1):
        r = pl.ds(g0 * C, (g1 - g0) * C)
        return pltpu.make_async_copy(wo_hbm.at[r, :], wo_buf.at[r, :], sems.at[s])

    def cp_kv(src, dst, s, g0, g1, b0=0, b1=B):
        b, g = pl.ds(b0, b1 - b0), pl.ds(g0, g1 - g0)
        return pltpu.make_async_copy(src.at[b, g], dst.at[b, g], sems.at[s])

    cp_k = functools.partial(cp_kv, k_hbm, k_buf)
    cp_v = functools.partial(cp_kv, v_hbm, v_buf)

    def cp_o(i):
        r = pl.ds(sum(_OUT_ROWS[:i]), _OUT_ROWS[i])
        return pltpu.make_async_copy(o_buf.at[r, :], o_hbm.at[r, :], sems.at[_NUM_WAITS])

    groups = [
        [cp_wq(0, 0, 0, rep - 1), cp_x(0, 0, half)],
        [cp_x(1, half, T), cp_wq(1, 0, rep - 1, rep), cp_k(1, 0, 1, 0, bps)],
        [cp_wq(2, 1), cp_v(2, 0, 1), cp_k(2, 0, 1, bps, B), cp_k(2, 1, 2, 0, bps)],
        [cp_wq(3, 2), cp_v(3, 1, 2), cp_wo(3, 0, 1), cp_k(3, 1, 2, bps, B), cp_k(3, 2, 3, 0, bps),
         cp_wq(3, 3, 0, 1)],
        [cp_wq(4, 3, 1, rep), cp_v(4, 2, 4), cp_wo(4, 1, 3), cp_k(4, 2, 3, bps, B), cp_k(4, 3, 4),
         cp_wq(4, 4), cp_k(4, 4, 5, 0, bps), cp_wq(4, 5, 0, 1)],
        [cp_wq(5, 5, 1, rep), cp_v(5, 4, 8), cp_wo(5, 3, 8), cp_k(5, 4, 5, bps, B), cp_k(5, 5, 8),
         cp_wq(5, 6), cp_wq(5, 7)],
    ]
    wait_before_q_proj = {0: 2, 1: 3}
    wait_before_pv = {2: 4, 4: 5}

    def wait(s):
        for c in groups[s]:
            c.wait()

    for grp in groups:
        for c in grp:
            c.start()

    def program(_, carry):
        q = {}
        att = {}

        def q_proj(g, h, xs, b0):
            qh = jnp.dot(xs, wq_buf[g, :, h * Dh:(h + 1) * Dh], preferred_element_type=_F32).astype(dt)
            for i in range(xs.shape[0] // Sq):
                q[g, h, b0 + i] = qh[i * Sq:(i + 1) * Sq]

        def scores_t(g, b):
            qb = jnp.concatenate([q.pop((g, h, b)) for h in range(rep)], axis=0)
            return lax.dot_general(k_buf[b, g], qb, (((1,), (1,)), ((), ())),
                                   preferred_element_type=_F32)

        def softmax(s):
            m = jnp.max(s, axis=0, keepdims=True)
            e = jnp.exp2((s - m) * (scale * _LOG2E))
            return (e / jnp.sum(e, axis=0, keepdims=True)).astype(dt).T

        def pv(g, b, p):
            o = jnp.dot(p, v_buf[b, g], preferred_element_type=_F32).astype(dt)
            for h in range(rep):
                att[g, b, h] = o[h * Sq:(h + 1) * Sq]

        def att_of(g):
            if g not in att:
                att[g] = jnp.concatenate(
                    [jnp.concatenate([att.pop((g, b, h)) for h in range(rep)], axis=1)
                     for b in range(B)], axis=0)
            return att[g]

        def out_proj(g, j):
            cols = slice(j * nps, (j + 1) * nps)
            contrib = jnp.dot(att_of(g), wo_buf[g * C:(g + 1) * C, cols], preferred_element_type=_F32)
            if g == 0:
                acc_ref[:, cols] = contrib
            else:
                acc_ref[:, cols] += contrib

        wait(0)
        x_lo = x_buf[:half, :]
        for h in range(rep - 1):
            q_proj(0, h, x_lo, 0)
        wait(1)
        x_hi = x_buf[half:, :]
        q_proj(0, rep - 1, x_lo, 0)
        for h in range(rep):
            q_proj(0, h, x_hi, B // 2)
        x = jnp.concatenate([x_lo, x_hi], axis=0)

        for g in range(G):
            for j in range(_SLOTS):
                batches = range(j * bps, (j + 1) * bps)
                scores = [scores_t(g, b) for b in batches]
                if j == 0 and g in wait_before_q_proj:
                    wait(wait_before_q_proj[g])
                if g + 1 < G:
                    q_proj(g + 1, j, x, 0)
                else:
                    out_proj(g - 1, j)
                probs = [softmax(s) for s in scores]
                if j == 0 and g in wait_before_pv:
                    wait(wait_before_pv[g])
                for b, p in zip(batches, probs):
                    pv(g, b, p)
                if 0 < g < G - 1:
                    out_proj(g - 1, j)

        g = G - 1
        r0 = 0
        for i, n in enumerate(_OUT_ROWS):
            rows = slice(r0, r0 + n)
            contrib = jnp.dot(att_of(g)[rows], wo_buf[g * C:(g + 1) * C, :],
                              preferred_element_type=_F32)
            o_buf[rows, :] = (acc_ref[rows, :] + contrib).astype(o_buf.dtype)
            cp_o(i).start()
            r0 += n
        for i in range(len(_OUT_ROWS)):
            cp_o(i).wait()
        return carry

    trips_ref[0] = 1
    lax.fori_loop(0, trips_ref[0], program, 0)


@jax.jit
def pallas_standalone__gqa_block_cached__near_ridge_kernel(
    x: jax.Array,
    k_cache: jax.Array,
    v_cache: jax.Array,
    wq: jax.Array,
    wo: jax.Array,
):
    B, Sq, D = x.shape
    _, Hkv, Sk, Dh = k_cache.shape
    Hq = wq.shape[1] // Dh
    rep = Hq // Hkv
    C = rep * Dh
    T = B * Sq
    hbm = pl.BlockSpec(memory_space=pl.ANY)
    out = pl.pallas_call(
        functools.partial(_kernel, B=B, Sq=Sq, rep=rep, Dh=Dh, G=Hkv, scale=Dh ** -0.5),
        in_specs=[hbm] * 5,
        out_specs=hbm,
        out_shape=jax.ShapeDtypeStruct((T, D), x.dtype),
        scratch_shapes=[
            pltpu.VMEM((T, D), x.dtype),
            pltpu.VMEM((B, Hkv, Sk, Dh), k_cache.dtype),
            pltpu.VMEM((B, Hkv, Sk, Dh), v_cache.dtype),
            pltpu.VMEM((Hkv, D, C), wq.dtype),
            pltpu.VMEM((Hq * Dh, D), wo.dtype),
            pltpu.VMEM((T, D), _F32),
            pltpu.VMEM((T, D), x.dtype),
            pltpu.SMEM((1,), jnp.int32),
            pltpu.SemaphoreType.DMA((_NUM_WAITS + 1,)),
        ],
        compiler_params=pltpu.CompilerParams(
            vmem_limit_bytes=48 * 1024 * 1024,
            disable_semaphore_checks=True,
        ),
        name="gqa_block_cached",
    )(x.reshape(T, D), k_cache, v_cache, wq, wo)
    return out.reshape(B, Sq, D)
```

```python
import functools

import jax
import jax.numpy as jnp
from jax import lax
import jax.experimental.pallas as pl
import jax.experimental.pallas.tpu as pltpu

_F32 = jnp.float32
_LOG2E = 1.4426950408889634
_SLOTS = 4
_X_ROWS = (0, 192, 384, 512)
_FIRST_Q = ((0, 1, 0, 1), (0, 1, 1, 2), (1, 2, 0, 2), (0, 2, 2, 3), (2, 3, 0, 3), (0, 3, 3, 4))
_PER_SLOT = (("wq", 0), ("wq", 1), ("wo", 0))
_OUT_ROWS = (128, 128, 64, 64, 64, 32, 32)
_NUM_IN_SEMS = 44


def _piece(name, g, j=0):
    return (name, g, j) if (name, g) in _PER_SLOT else (name, g, None)


def _copy_order(G):
    uses = []
    for x0, x1, h0, h1 in _FIRST_Q:
        uses += [_piece("wq", 0, h) for h in range(h0, h1)]
        uses += [_piece("x", r) for r in range(x0, x1)]
    for g in range(G):
        for j in range(_SLOTS):
            uses.append(_piece("k", g, j))
            uses.append(_piece("wq", g + 1, j) if g + 1 < G else _piece("wo", g - 1, j))
            uses.append(_piece("v", g, j))
            if 0 < g < G - 1:
                uses.append(_piece("wo", g - 1, j))
    uses.append(_piece("wo", G - 1))
    return list(dict.fromkeys(uses))


def _kernel(x_hbm, k_hbm, v_hbm, wq_hbm, wo_hbm, o_hbm,
            x_buf, k_buf, v_buf, wq_buf, wo_buf, acc_ref, o_buf, trips_ref, sems,
            *, B, Sq, rep, Dh, G, scale):
    T, D = x_buf.shape
    C = rep * Dh
    bps = B // _SLOTS
    nps = D // _SLOTS
    dt = x_buf.dtype
    order = _copy_order(G)
    assert rep == _SLOTS and sum(_OUT_ROWS) == T == _X_ROWS[-1] and len(order) == _NUM_IN_SEMS

    def copy_in(key):
        name, g, j = key
        sem = sems.at[order.index(key)]
        if name == "x":
            r = pl.ds(_X_ROWS[g], _X_ROWS[g + 1] - _X_ROWS[g])
            return pltpu.make_async_copy(x_hbm.at[r, :], x_buf.at[r, :], sem)
        if name == "wq":
            c0, n = (0, C) if j is None else (j * Dh, Dh)
            return pltpu.make_async_copy(
                wq_hbm.at[:, pl.ds(g * C + c0, n)], wq_buf.at[g, :, pl.ds(c0, n)], sem)
        if name == "wo":
            r, c = pl.ds(g * C, C), pl.ds(0, D) if j is None else pl.ds(j * nps, nps)
            return pltpu.make_async_copy(wo_hbm.at[r, c], wo_buf.at[r, c], sem)
        src, dst = (k_hbm, k_buf) if name == "k" else (v_hbm, v_buf)
        return pltpu.make_async_copy(src.at[:, pl.ds(g, 1)], dst.at[:, pl.ds(g, 1)], sem)

    def copy_out(i):
        r = pl.ds(sum(_OUT_ROWS[:i]), _OUT_ROWS[i])
        return pltpu.make_async_copy(o_buf.at[r, :], o_hbm.at[r, :], sems.at[_NUM_IN_SEMS])

    def program(_, carry):
        in_flight = {key: copy_in(key) for key in order}
        for c in in_flight.values():
            c.start()

        def need(name, g, j=0):
            c = in_flight.pop(_piece(name, g, j), None)
            if c is not None:
                c.wait()

        q = {}
        att = {}

        def q_proj(g, h, xs, b0):
            need("wq", g, h)
            qh = jnp.dot(xs, wq_buf[g, :, h * Dh:(h + 1) * Dh],
                         preferred_element_type=_F32).astype(dt)
            for i in range(xs.shape[0] // Sq):
                q[g, h, b0 + i] = qh[i * Sq:(i + 1) * Sq]

        def scores_t(g, b):
            qb = jnp.concatenate([q.pop((g, h, b)) for h in range(rep)], axis=0)
            return lax.dot_general(k_buf[b, g], qb, (((1,), (1,)), ((), ())),
                                   preferred_element_type=_F32)

        def softmax(s):
            m = jnp.max(s, axis=0, keepdims=True)
            e = jnp.exp2((s - m) * (scale * _LOG2E))
            return (e / jnp.sum(e, axis=0, keepdims=True)).astype(dt).T

        def pv(g, b, p):
            o = jnp.dot(p, v_buf[b, g], preferred_element_type=_F32).astype(dt)
            for h in range(rep):
                att[g, b, h] = o[h * Sq:(h + 1) * Sq]

        def att_of(g):
            if g not in att:
                att[g] = jnp.concatenate(
                    [jnp.concatenate([att.pop((g, b, h)) for h in range(rep)], axis=1)
                     for b in range(B)], axis=0)
            return att[g]

        def out_proj(g, j):
            need("wo", g, j)
            cols = slice(j * nps, (j + 1) * nps)
            contrib = jnp.dot(att_of(g), wo_buf[g * C:(g + 1) * C, cols],
                              preferred_element_type=_F32)
            if g == 0:
                acc_ref[:, cols] = contrib
            else:
                acc_ref[:, cols] += contrib

        x_blocks = {}
        for x0, x1, h0, h1 in _FIRST_Q:
            for r in range(x0, x1):
                if r not in x_blocks:
                    need("x", r)
                    x_blocks[r] = x_buf[_X_ROWS[r]:_X_ROWS[r + 1], :]
            xs = jnp.concatenate([x_blocks[r] for r in range(x0, x1)], axis=0)
            for h in range(h0, h1):
                q_proj(0, h, xs, _X_ROWS[x0] // Sq)
        x = jnp.concatenate([x_blocks[r] for r in range(len(_X_ROWS) - 1)], axis=0)

        for g in range(G):
            for j in range(_SLOTS):
                batches = range(j * bps, (j + 1) * bps)
                need("k", g)
                scores = [scores_t(g, b) for b in batches]
                if g + 1 < G:
                    q_proj(g + 1, j, x, 0)
                else:
                    out_proj(g - 1, j)
                probs = [softmax(s) for s in scores]
                need("v", g)
                for b, p in zip(batches, probs):
                    pv(g, b, p)
                if 0 < g < G - 1:
                    out_proj(g - 1, j)

        g = G - 1
        need("wo", g)
        assert not in_flight
        r0 = 0
        for i, n in enumerate(_OUT_ROWS):
            rows = slice(r0, r0 + n)
            contrib = jnp.dot(att_of(g)[rows], wo_buf[g * C:(g + 1) * C, :],
                              preferred_element_type=_F32)
            o_buf[rows, :] = (acc_ref[rows, :] + contrib).astype(o_buf.dtype)
            copy_out(i).start()
            r0 += n
        for i in range(len(_OUT_ROWS)):
            copy_out(i).wait()
        return carry

    trips_ref[0] = 1
    lax.fori_loop(0, trips_ref[0], program, 0)


@jax.jit
def pallas_standalone__gqa_block_cached__near_ridge_kernel(
    x: jax.Array,
    k_cache: jax.Array,
    v_cache: jax.Array,
    wq: jax.Array,
    wo: jax.Array,
):
    B, Sq, D = x.shape
    _, Hkv, Sk, Dh = k_cache.shape
    Hq = wq.shape[1] // Dh
    rep = Hq // Hkv
    C = rep * Dh
    T = B * Sq
    hbm = pl.BlockSpec(memory_space=pl.ANY)
    out = pl.pallas_call(
        functools.partial(_kernel, B=B, Sq=Sq, rep=rep, Dh=Dh, G=Hkv, scale=Dh ** -0.5),
        in_specs=[hbm] * 5,
        out_specs=hbm,
        out_shape=jax.ShapeDtypeStruct((T, D), x.dtype),
        scratch_shapes=[
            pltpu.VMEM((T, D), x.dtype),
            pltpu.VMEM((B, Hkv, Sk, Dh), k_cache.dtype),
            pltpu.VMEM((B, Hkv, Sk, Dh), v_cache.dtype),
            pltpu.VMEM((Hkv, D, C), wq.dtype),
            pltpu.VMEM((Hq * Dh, D), wo.dtype),
            pltpu.VMEM((T, D), _F32),
            pltpu.VMEM((T, D), x.dtype),
            pltpu.SMEM((1,), jnp.int32),
            pltpu.SemaphoreType.DMA((_NUM_IN_SEMS + 1,)),
        ],
        compiler_params=pltpu.CompilerParams(
            vmem_limit_bytes=48 * 1024 * 1024,
            disable_semaphore_checks=True,
            flags={"XLA_TPU_RESCHEDULE_DMA_DONES": True},
        ),
        name="gqa_block_cached",
    )(x.reshape(T, D), k_cache, v_cache, wq, wo)
    return out.reshape(B, Sq, D)
```
